```python
import jax
import jax.numpy as jnp

def _softmax(x, axis=-1):
    return jax.nn.softmax(x, axis=axis)
def _gelu(x):
    return jax.nn.gelu(x, approximate=True)
def _silu(x):
    return jax.nn.silu(x)
def _sigmoid(x):
    return jax.nn.sigmoid(x)
def _layernorm(x, axis=-1, eps=1e-5):
    m = jnp.mean(x, axis=axis, keepdims=True)
    v = jnp.var(x, axis=axis, keepdims=True)
    return (x - m) / jnp.sqrt(v + eps)
def _scatter_add(tgt, idx, src, axis=0):
    return tgt.at[idx].add(src)
def _segment_sum(src, seg, n):
    return jax.ops.segment_sum(src, seg, n)
class _Rng:
    def __init__(self, key):
        self._k = key
    def _next(self):
        self._k, sub = jax.random.split(self._k)
        return sub
    def normal(self, shape):
        return jax.random.normal(self._next(), shape, dtype=jnp.bfloat16)
    def randint(self, lo, hi, shape):
        return jax.random.randint(self._next(), shape, lo, hi, dtype=jnp.int32)
    def uniform(self, shape, lo=0.0, hi=1.0):
        return jax.random.uniform(self._next(), shape, jnp.bfloat16, lo, hi)
    def permutation(self, n):
        return jax.random.permutation(self._next(), n)


kernel_name = 'parallel_sum__sliding_block_cached__mixer_s_mlp__decode'

def setup_inputs():
    _rng = _Rng(jax.random.key(int.from_bytes(__import__("os").urandom(4), "little")))
    _w = (lambda a: (lambda t: t.astype(jnp.bfloat16) if jnp.issubdtype(t.dtype, jnp.floating) else t)(jnp.asarray(a)))
    def _A_setup():
        B, Sq, D = 4, 1, 512
        Hq, Hkv, Sk, Dh = 32, 32, 8192, 128
        assert Hq % Hkv == 0, (Hq, Hkv)
        return {
            "x": _w((lambda *s: _rng.normal(s) * 0.05)(B, Sq, D)),
            "k_cache": _w((lambda *s: _rng.normal(s) * 0.05)(B, Hkv, Sk, Dh)),
            "v_cache": _w((lambda *s: _rng.normal(s) * 0.05)(B, Hkv, Sk, Dh)),
            "wq": _w((lambda *s: _rng.normal(s) * 0.05)(D, Hq * Dh) * (D ** -0.5)),
            "wo": _w((lambda *s: _rng.normal(s) * 0.05)(Hq * Dh, D) * ((Hq * Dh) ** -0.5)),
        }
    _A_in = _A_setup()

    def _B_setup():
        B, S, D, F = 4, 1, 512, 1376
        return {
            "x":  _w((lambda *s: _rng.normal(s) * 0.05)(B, S, D)),
            "w1": _w((lambda *s: _rng.normal(s) * 0.05)(D, D) * (D ** -0.5)),
            "w2": _w((lambda *s: _rng.normal(s) * 0.05)(D, D) * (D ** -0.5)),
            "w3": _w((lambda *s: _rng.normal(s) * 0.05)(D, F) * (D ** -0.5)),
            "w4": _w((lambda *s: _rng.normal(s) * 0.05)(F, D) * (F ** -0.5)),
        }
    _B_in = _B_setup()

    return {
        "A_x": _A_in["x"],
        "A_k_cache": _A_in["k_cache"],
        "A_v_cache": _A_in["v_cache"],
        "A_wq": _A_in["wq"],
        "A_wo": _A_in["wo"],
        "B_x": _B_in["x"],
        "B_w1": _B_in["w1"],
        "B_w2": _B_in["w2"],
        "B_w3": _B_in["w3"],
        "B_w4": _B_in["w4"],
    }

def reference(A_x, A_k_cache, A_v_cache, A_wq, A_wo, B_x, B_w1, B_w2, B_w3, B_w4):
    def _A_ref(x, k_cache, v_cache, wq, wo):
        B, Sq, D = x.shape
        Hq, Dh = 32, 128
        Hkv, Sk = k_cache.shape[1], k_cache.shape[2]
        W = min(4096, max(256, Sk // 4))
        rep = Hq // Hkv
        q = (lambda x, *d: x.transpose(*d))((x @ wq).reshape(B, Sq, Hq, Dh), 0, 2, 1, 3)
        k = jnp.repeat(k_cache[:, :, Sk - W:, :], rep, axis=1)
        v = jnp.repeat(v_cache[:, :, Sk - W:, :], rep, axis=1)
        scores = jnp.einsum("bhqd,bhkd->bhqk", q, k) * (Dh ** -0.5)
        p = _softmax(scores, axis=-1)
        o = jnp.einsum("bhqk,bhkd->bhqd", p, v)
        return (lambda x, *d: x.transpose(*d))(o, 0, 2, 1, 3).reshape(B, Sq, Hq * Dh) @ wo

    def _B_ref(x, w1, w2, w3, w4):
        B, S, D = x.shape
        h = _gelu(_layernorm(x, axis=-1) @ w1)
        c = D // 4
        g0 = jnp.pad(h[:, :, 0*c:1*c], ((0, 0), (1, 0), (0, 0)))[:, :S, :]
        g1 = jnp.pad(h[:, :, 1*c:2*c], ((0, 0), (0, 1), (0, 0)))[:, 1:, :]
        g2 = jnp.pad(h[:, :, 2*c:3*c], ((0, 0), (2, 0), (0, 0)))[:, :S, :]
        g3 = jnp.pad(h[:, :, 3*c:   ], ((0, 0), (0, 2), (0, 0)))[:, 2:, :]
        hs = jnp.concatenate([g0, g1, g2, g3], axis=-1) @ w2
        x1 = x + hs
        h2 = _gelu(_layernorm(x1, axis=-1) @ w3) @ w4
        return x1 + h2

    x = A_x
    xn = _layernorm(x, axis=-1)
    return x + _A_ref(xn, A_k_cache, A_v_cache, A_wq, A_wo) + _B_ref(xn, B_w1, B_w2, B_w3, B_w4)
```

```python
import functools
import jax
import jax.numpy as jnp
from jax import lax
from jax.experimental import pallas as pl
from jax.experimental.pallas import tpu as pltpu

_NT = (((1,), (1,)), ((), ()))
_NN = (((1,), (0,)), ((), ()))


def _layernorm(x, eps=1e-5):
    m = jnp.mean(x, axis=-1, keepdims=True)
    d = x - m
    v = jnp.mean(d * d, axis=-1, keepdims=True)
    return d / jnp.sqrt(v + eps)


def make(UR=256, LOOK=4, PR=64, WQC=32, tail_rows=None, prio=(0, 1)):
    def f(A_x, A_k_cache, A_v_cache, A_wq, A_wo, B_x, B_w1, B_w2, B_w3, B_w4):
        B, _, D = A_x.shape
        _, H, SK, DH = A_k_cache.shape
        F = B_w3.shape[1]
        W = min(4096, max(256, SK // 4))
        HG = 2
        NG = H // HG
        NU = W // UR
        scale = DH ** -0.5
        f32, bf16 = jnp.float32, jnp.bfloat16

        def kern(x_hbm, k_hbm, v_hbm, wq_hbm, wo_hbm, w3t_hbm, w4_hbm, o_ref,
                 x_buf, kv_buf, wq_buf, wo_buf, w3_buf, w4_buf, q_buf, a_buf, kv_sem, w_sem):
            cnt = [0]
            def go(src, dst, sem):
                pltpu.make_async_copy(src, dst, sem).start(priority=prio[cnt[0] % len(prio)])
                cnt[0] += 1
            def wait(dst, sem):
                pltpu.make_async_copy(dst, dst, sem).wait()

            def kv_start(g, u):
                src = k_hbm if u < NU else v_hbm
                for r in range(UR // PR):
                    for b in range(B):
                        go(src.at[b, pl.ds(g * HG, HG), pl.ds(SK - W + (u % NU) * UR + r * PR, PR), :],
                           kv_buf.at[u, b, :, pl.ds(r * PR, PR), :], kv_sem.at[u])
            def rows_start(src, dst, r0, n, piece, sem):
                for r in range(r0, r0 + n, piece):
                    m = min(piece, r0 + n - r)
                    go(src.at[pl.ds(r, m), :], dst.at[pl.ds(r, m), :], sem)
            def wq_start(i, sem):
                for r in range(i * 64, (i + 1) * 64, 8):
                    for c in range(2):
                        go(wq_hbm.at[pl.ds(r, 8), pl.ds(c * 2048, 2048)], wq_buf.at[pl.ds(r, 8), pl.ds(c * 2048, 2048)], sem)

            f_units = [(r, min(512, F - r)) for r in range(0, F, 512)]
            head = []
            for (r, n) in f_units:
                head.append(functools.partial(rows_start, w3t_hbm, w3_buf, r, n, 32))
            for (r, n) in f_units:
                head.append(functools.partial(rows_start, w4_hbm, w4_buf, r, n, 32))
            for i in range(D // 64):
                head.append(functools.partial(wq_start, i))
            NH = len(head)
            wo_units = tail_rows or [512] * (H * DH // 512)
            wo_off = [sum(wo_units[:i]) for i in range(len(wo_units))]
            NT = len(wo_units)

            def issue_head(i):
                if i < NH:
                    head[i](w_sem.at[i])
                else:
                    kv_start(0, i - NH)
            def issue_tail(i):
                if i < NT:
                    rows_start(wo_hbm, wo_buf, wo_off[i], wo_units[i], 32, w_sem.at[NH + i])

            xc = pltpu.make_async_copy(x_hbm, x_buf, w_sem.at[NH + NT])
            xc.start()
            for i in range(LOOK):
                issue_head(i)
            xc.wait()
            x4 = x_buf[...].astype(f32)
            x = jnp.concatenate([x4, x4], axis=0)
            xn = _layernorm(x).astype(bf16)
            xn2 = _layernorm(xn.astype(f32)).astype(bf16)
            step = 0
            hs = []
            for (r, n) in f_units:
                wait(w3_buf.at[pl.ds(r, n), :], w_sem.at[step]); issue_head(step + LOOK); step += 1
                h = lax.dot_general(xn2, w3_buf[pl.ds(r, n), :], _NT, preferred_element_type=f32)
                hs.append(jax.nn.gelu(h, approximate=True).astype(bf16))
            res = x + xn.astype(f32)
            for h, (r, n) in zip(hs, f_units):
                wait(w4_buf.at[pl.ds(r, n), :], w_sem.at[step]); issue_head(step + LOOK); step += 1
                res = res + lax.dot_general(h, w4_buf[pl.ds(r, n), :], _NN, preferred_element_type=f32)
            q = None
            for i in range(D // 64):
                wait(wq_buf.at[pl.ds(i * 64, 64), :], w_sem.at[step]); issue_head(step + LOOK); step += 1
                if i % 2 == 1:
                    c = (i // 2) * 128
                    t = lax.dot_general(xn[:, c:c + 128], wq_buf[pl.ds(c, 128), :], _NN, preferred_element_type=f32)
                    q = t if q is None else q + t
            row = lax.broadcasted_iota(jnp.int32, (HG * B, DH), 0)
            for g in range(NG):
                q_buf[g] = jnp.where(row < B, q[:, (2 * g) * DH:(2 * g + 1) * DH], q[:, (2 * g + 1) * DH:(2 * g + 2) * DH])

            def group(g, last):
                def issue(u):
                    if u < 2 * NU:
                        kv_start(g, u)
                    elif last:
                        issue_tail(u - 2 * NU)
                    else:
                        kv_start(g + 1, u - 2 * NU)
                qg = q_buf[g].astype(bf16)
                rowu = lax.broadcasted_iota(jnp.int32, (HG * B, UR), 0)
                ss = []
                for u in range(NU):
                    wait(kv_buf.at[u], kv_sem.at[u]); issue(u + LOOK)
                    s = None
                    for hh in range(HG):
                        for b in range(B):
                            t = lax.dot_general(qg, kv_buf[u, b, hh], _NT, preferred_element_type=f32)
                            s = t if s is None else jnp.where(rowu == hh * B + b, t, s)
                    ss.append(s * scale)
                m = functools.reduce(jnp.maximum, ss)
                m = jnp.max(m, axis=-1, keepdims=True)
                ps = [jnp.exp(s - m) for s in ss]
                l = jnp.sum(functools.reduce(jnp.add, ps), axis=-1, keepdims=True)
                acc = [None] * (HG * B)
                for u in range(NU):
                    wait(kv_buf.at[NU + u], kv_sem.at[NU + u]); issue(NU + u + LOOK)
                    p = ps[u].astype(bf16)
                    for hh in range(HG):
                        for b in range(B):
                            t = lax.dot_general(p, kv_buf[NU + u, b, hh], _NN, preferred_element_type=f32)
                            j = hh * B + b
                            acc[j] = t if acc[j] is None else acc[j] + t
                o = acc[0]
                for j in range(1, HG * B):
                    o = jnp.where(row == j, acc[j], o)
                a_buf[g] = o / l

            def body(g, c):
                group(g, False)
                return c
            lax.fori_loop(0, NG - 1, body, 0)
            group(NG - 1, True)

            out = None
            for i in range(NT):
                lhs = []
                for h in range(wo_off[i] // DH, (wo_off[i] + wo_units[i]) // DH):
                    a = a_buf[h // HG]
                    keep = (row < B) if h % HG == 0 else (row >= B)
                    lhs.append(jnp.where(keep, a, 0.0).astype(bf16))
                lhs = jnp.concatenate(lhs, axis=1)
                wait(wo_buf.at[pl.ds(wo_off[i], wo_units[i]), :], w_sem.at[NH + i]); issue_tail(i + LOOK)
                t = lax.dot_general(lhs, wo_buf[pl.ds(wo_off[i], wo_units[i]), :], _NN, preferred_element_type=f32)
                out = t if out is None else out + t
            o_ref[...] = (res[0:B] + out[0:B] + out[B:2 * B]).astype(o_ref.dtype)

        hbm = pl.BlockSpec(memory_space=pltpu.HBM)
        out = pl.pallas_call(
            kern,
            in_specs=[hbm] * 7,
            out_specs=pl.BlockSpec(memory_space=pltpu.VMEM),
            out_shape=jax.ShapeDtypeStruct((B, D), A_x.dtype),
            scratch_shapes=[
                pltpu.VMEM((B, D), bf16),
                pltpu.VMEM((2 * NU, B, HG, UR, DH), bf16),
                pltpu.VMEM((D, H * DH), bf16),
                pltpu.VMEM((H * DH, D), bf16),
                pltpu.VMEM((F, D), bf16),
                pltpu.VMEM((F, D), bf16),
                pltpu.VMEM((NG, HG * B, DH), f32),
                pltpu.VMEM((NG, HG * B, DH), f32),
                pltpu.SemaphoreType.DMA((2 * NU,)),
                pltpu.SemaphoreType.DMA((64,)),
            ],
            compiler_params=pltpu.CompilerParams(vmem_limit_bytes=64 * 2**20, disable_bounds_checks=True),
        )(A_x.reshape(B, D), A_k_cache, A_v_cache, A_wq, A_wo, B_w3.T, B_w4)
        return out.reshape(B, 1, D)
    return f


_kernel_impl = make(UR=256, LOOK=6)


@jax.jit
def pallas_parallel_sum__sliding_block_cached__mixer_s_mlp__decode_kernel(
    A_x, A_k_cache, A_v_cache, A_wq, A_wo, B_x, B_w1, B_w2, B_w3, B_w4,
):
    return _kernel_impl(A_x, A_k_cache, A_v_cache, A_wq, A_wo, B_x, B_w1, B_w2, B_w3, B_w4)
```

```python
import functools
import jax
import jax.numpy as jnp
from jax import lax
from jax.experimental import pallas as pl
from jax.experimental.pallas import tpu as pltpu

_NT = (((1,), (1,)), ((), ()))
_NN = (((1,), (0,)), ((), ()))


def _layernorm(x, eps=1e-5):
    m = jnp.mean(x, axis=-1, keepdims=True)
    d = x - m
    v = jnp.mean(d * d, axis=-1, keepdims=True)
    return d / jnp.sqrt(v + eps)


def _loop(lo, hi, fn):
    def body(i, c):
        fn(i)
        return c
    lax.fori_loop(lo, hi, body, 0)


def make(UR=128, LOOK=8, PR=64, prio=(0, 1), pre=None, nocompute=False, wq_str=True, wo_str=True, mlp_p=(1, 1), mlp_str=True):
    def f(A_x, A_k_cache, A_v_cache, A_wq, A_wo, B_x, B_w1, B_w2, B_w3, B_w4):
        B, _, D = A_x.shape
        _, H, SK, DH = A_k_cache.shape
        F = B_w3.shape[1]
        W = min(4096, max(256, SK // 4))
        HG = 16
        NG = B * H // HG
        NU = W // UR
        PRE = LOOK // 2 if pre is None else pre
        scale = DH ** -0.5
        f32, bf16 = jnp.float32, jnp.bfloat16
        NO = 4

        def kern(x_hbm, k_hbm, v_hbm, wq_hbm, wo_hbm, w3t_hbm, w4_hbm, o_ref,
                 x_buf, k_buf, v_buf, wq_buf, wo_buf, w3_buf, w4_buf, q_buf, a_buf, s_buf, k_sem, v_sem, w_sem, o_sem):
            def go(src, dst, sem, p):
                pltpu.make_async_copy(src, dst, sem).start(priority=p)
            def wait(dst, sem):
                pltpu.make_async_copy(dst, dst, sem).wait()

            def kv_start(src, buf, sem, g, u):
                i = 0
                for r in range(0, UR, PR):
                    r0 = pl.multiple_of(SK - W + u * UR + r, PR)
                    for j in range(0, HG, 2):
                        go(src.at[pl.ds(g * HG + j, 2), pl.ds(r0, PR), :], buf.at[u, pl.ds(j, 2), pl.ds(r, PR), :], sem.at[u], prio[i % len(prio)]); i += 1
            def wo_start(u):
                n = 128 // LOOK
                for i in range(n):
                    t = u * n + i
                    if wo_str:
                        s, o, r = t % 8, t // 32, (t // 8) % 4
                    else:
                        s, o, r = (t // 4) % 8, t // 32, t % 4
                    r0 = pl.multiple_of(r * 32, 32)
                    h = s * NO + o if wo_str else o * 8 + s
                    go(wo_hbm.at[pl.ds(pl.multiple_of(h * DH + r0, 32), 32), :], wo_buf.at[o, s, pl.ds(r0, 32), :], o_sem.at[o], prio[i % len(prio)])

            xc = pltpu.make_async_copy(x_hbm, x_buf, w_sem.at[0])
            xc.start()
            NF = F // 32
            def mlp_w(i):
                r0 = pl.multiple_of((lax.rem(i * 16, NF) if mlp_str else i) * 32, 32)
                go(w3t_hbm.at[pl.ds(r0, 32), :], w3_buf.at[pl.ds(r0, 32), :], w_sem.at[1], mlp_p[0])
                go(w4_hbm.at[pl.ds(r0, 32), :], w4_buf.at[pl.ds(r0, 32), :], w_sem.at[2], mlp_p[1])
            _loop(0, NF, mlp_w)
            def q_w(i):
                if wq_str:
                    c0 = pl.multiple_of((i % 2) * 2048, 2048)
                    for s in range(8):
                        r0 = pl.multiple_of(s * 64 + (i // 2) * 8, 8)
                        go(wq_hbm.at[pl.ds(r0, 8), pl.ds(c0, 2048)], wq_buf.at[pl.ds(r0, 8), pl.ds(c0, 2048)], w_sem.at[3], prio[s % len(prio)])
                else:
                    for s in range(8):
                        r0 = pl.multiple_of(i * 32 + (s // 2) * 8, 8)
                        go(wq_hbm.at[pl.ds(r0, 8), pl.ds((s % 2) * 2048, 2048)], wq_buf.at[pl.ds(r0, 8), pl.ds((s % 2) * 2048, 2048)], w_sem.at[3], prio[s % len(prio)])
            _loop(0, 16, q_w)

            xc.wait()
            x4 = x_buf[...].astype(f32)
            x = jnp.concatenate([x4, x4], axis=0)
            xn = _layernorm(x).astype(bf16)
            xn2 = _layernorm(xn.astype(f32)).astype(bf16)
            a_buf[...] = jnp.zeros_like(a_buf)
            wait(w3_buf, w_sem.at[1])
            wait(w4_buf, w_sem.at[2])
            h = lax.dot_general(xn2, w3_buf[...], _NT, preferred_element_type=f32)
            h = jax.nn.gelu(h, approximate=True).astype(bf16)
            res = x + xn.astype(f32) + lax.dot_general(h, w4_buf[...], _NN, preferred_element_type=f32)

            _loop(0, PRE, lambda u: kv_start(k_hbm, k_buf, k_sem, 0, u))
            wait(wq_buf, w_sem.at[3])
            QS = LOOK - PRE if LOOK > PRE else 8
            QH = H // QS
            def q_proj(i):
                if LOOK > PRE:
                    kv_start(k_hbm, k_buf, k_sem, 0, PRE + i)
                c0 = pl.multiple_of(i * QH * DH, QH * DH)
                q = lax.dot_general(xn, wq_buf[:, pl.ds(c0, QH * DH)], _NN, preferred_element_type=f32)
                for j in range(QH):
                    q_buf[pl.ds(pl.multiple_of((i * QH + j) * 8, 8), 8), :] = q[:, j * DH:(j + 1) * DH]
            _loop(0, QS, q_proj)

            row = lax.broadcasted_iota(jnp.int32, (8, DH), 0)
            rowu = lax.broadcasted_iota(jnp.int32, (8, UR), 0)
            def group(g):
                r0 = (g % (H // HG)) * (HG * 8) + g // (H // HG)
                qg = [q_buf[pl.ds(r0 + half * 64, 8, stride=8), :].astype(bf16) for half in range(2)]
                def k_step(issue, u, m):
                    wait(k_buf.at[u], k_sem.at[u])
                    issue(u)
                    if nocompute:
                        return m
                    ss = []
                    for half in range(2):
                        s = None
                        for j in range(8):
                            t = lax.dot_general(qg[half], k_buf[u, half * 8 + j], _NT, preferred_element_type=f32)
                            s = t if s is None else jnp.where(rowu == j, t, s)
                        ss.append(s * scale)
                    s = jnp.concatenate(ss, axis=0)
                    s_buf[u] = s
                    return jnp.maximum(m, s)
                m = jnp.full((HG, UR), -jnp.inf, f32)
                if NU > LOOK:
                    m = lax.fori_loop(0, NU - LOOK, functools.partial(k_step, lambda u: kv_start(k_hbm, k_buf, k_sem, g, u + LOOK)), m)
                m = lax.fori_loop(NU - LOOK, NU, functools.partial(k_step, lambda u: kv_start(v_hbm, v_buf, v_sem, g, u + LOOK - NU)), m)
                m = jnp.max(m, axis=-1, keepdims=True)
                def v_step(issue, u, c):
                    l, acc = c
                    wait(v_buf.at[u], v_sem.at[u])
                    issue(u)
                    if nocompute:
                        return c
                    p = jnp.exp(s_buf[u] - m)
                    os_ = []
                    for half in range(2):
                        ph = p[half * 8:(half + 1) * 8].astype(bf16)
                        o = None
                        for j in range(8):
                            t = lax.dot_general(ph, v_buf[u, half * 8 + j], _NN, preferred_element_type=f32)
                            o = t if o is None else jnp.where(row == j, t, o)
                        os_.append(o)
                    return l + p, acc + jnp.concatenate(os_, axis=0)
                def nxt(u):
                    pl.when(g < NG - 1)(lambda: kv_start(k_hbm, k_buf, k_sem, g + 1, u + LOOK - NU))
                    pl.when(g == NG - 1)(lambda: wo_start(u + LOOK - NU))
                c = (jnp.zeros((HG, UR), f32), jnp.zeros((HG, DH), f32))
                if NU > LOOK:
                    c = lax.fori_loop(0, NU - LOOK, functools.partial(v_step, lambda u: kv_start(v_hbm, v_buf, v_sem, g, u + LOOK)), c)
                l, acc = lax.fori_loop(NU - LOOK, NU, functools.partial(v_step, nxt), c)
                a_buf[pl.ds(r0, HG, stride=8), :] = acc / jnp.sum(l, axis=-1, keepdims=True)
            _loop(0, NG, group)

            def o_step(o, out):
                wait(wo_buf.at[o], o_sem.at[o])
                for s in range(8):
                    h = s * NO + o if wo_str else o * 8 + s
                    lhs = a_buf[pl.ds(pl.multiple_of(h * 8, 8), 8), :].astype(bf16)
                    out = out + lax.dot_general(lhs, wo_buf[o, s], _NN, preferred_element_type=f32)
                return out
            out = lax.fori_loop(0, NO, o_step, res)
            o_ref[...] = out[0:B].astype(o_ref.dtype)

        hbm = pl.BlockSpec(memory_space=pltpu.HBM)
        out = pl.pallas_call(
            kern,
            in_specs=[hbm] * 7,
            out_specs=pl.BlockSpec(memory_space=pltpu.VMEM),
            out_shape=jax.ShapeDtypeStruct((B, D), A_x.dtype),
            scratch_shapes=[
                pltpu.VMEM((B, D), bf16),
                pltpu.VMEM((NU, HG, UR, DH), bf16),
                pltpu.VMEM((NU, HG, UR, DH), bf16),
                pltpu.VMEM((D, H * DH), bf16),
                pltpu.VMEM((NO, 8, DH, D), bf16),
                pltpu.VMEM((F, D), bf16),
                pltpu.VMEM((F, D), bf16),
                pltpu.VMEM((H * 8, DH), f32),
                pltpu.VMEM((H * 8, DH), f32),
                pltpu.VMEM((NU, HG, UR), f32),
                pltpu.SemaphoreType.DMA((NU,)),
                pltpu.SemaphoreType.DMA((NU,)),
                pltpu.SemaphoreType.DMA((4,)),
                pltpu.SemaphoreType.DMA((NO,)),
            ],
            compiler_params=pltpu.CompilerParams(vmem_limit_bytes=64 * 2**20, disable_bounds_checks=True),
        )(A_x.reshape(B, D), A_k_cache.reshape(B * H, SK, DH), A_v_cache.reshape(B * H, SK, DH), A_wq, A_wo, B_w3.T, B_w4)
        return out.reshape(B, 1, D)
    return f


_kernel_impl = make(UR=256, LOOK=8)


@jax.jit
def pallas_parallel_sum__sliding_block_cached__mixer_s_mlp__decode_kernel(
    A_x, A_k_cache, A_v_cache, A_wq, A_wo, B_x, B_w1, B_w2, B_w3, B_w4,
):
    return _kernel_impl(A_x, A_k_cache, A_v_cache, A_wq, A_wo, B_x, B_w1, B_w2, B_w3, B_w4)
```

```python
import functools
import jax
import jax.numpy as jnp
from jax import lax
from jax.experimental import pallas as pl
from jax.experimental.pallas import tpu as pltpu

_NT = (((1,), (1,)), ((), ()))
_NN = (((1,), (0,)), ((), ()))


def _layernorm(x, eps=1e-5):
    m = jnp.mean(x, axis=-1, keepdims=True)
    d = x - m
    v = jnp.mean(d * d, axis=-1, keepdims=True)
    return d / jnp.sqrt(v + eps)


def _loop(lo, hi, fn):
    def body(i, c):
        fn(i)
        return c
    lax.fori_loop(lo, hi, body, 0)


def _ds(i, n):
    return pl.ds(pl.multiple_of(i * n, n), n)


def make(CR=128, NW=4, PR=64, nocompute=False, LAG=32, WS=4, head_mode=0, single=4, unroll=1, dsc=True, dbc=True):
    def f(A_x, A_k_cache, A_v_cache, A_wq, A_wo, B_x, B_w1, B_w2, B_w3, B_w4):
        B, _, D = A_x.shape
        _, H, SK, DH = A_k_cache.shape
        F = B_w3.shape[1]
        W = min(4096, max(256, SK // 4))
        HG = 16
        NG = B * H // HG
        NC = W // CR
        NP = W // PR
        F2 = F // 2
        FC = pl.cdiv(F2, 128)
        scale = DH ** -0.5
        f32, bf16 = jnp.float32, jnp.bfloat16

        def kern(x_hbm, k_hbm, v_hbm, wq_hbm, wo_hbm, w3t_hbm, w4_hbm, o_ref,
                 x_buf, k_buf, v_buf, wq_buf, wo_buf, w3_buf, w4_buf, q_buf, a_buf, s_buf, k_sem, v_sem, w_sem, o_sem):
            def go(src, dst, sem, p):
                pltpu.make_async_copy(src, dst, sem).start(priority=p)
            def wait(dst, sem):
                pltpu.make_async_copy(dst, dst, sem).wait()

            def kv_start(src, buf, sem, g, r):
                for j in range(0, HG, 2):
                    go(src.at[pl.ds(g * HG + j, 2), _ds((SK - W) // PR + r, PR), :], buf.at[pl.ds(j, 2), _ds(r, PR), :],
                       sem.at[lax.div(r, NP // NW)], (j // 2) % 2)
            def wo_pair(a, p, drain=False):
                k = a >> 5
                if drain:
                    j, r = (a >> 3) & 3, a & 7
                else:
                    j, r = a & 3, (a >> 2) & 7
                go(wo_hbm.at[_ds(j, 2), k, _ds(r, 16), :], wo_buf.at[_ds(j, 2), k, _ds(r, 16), :], o_sem.at[k * 2 + (j >> 1)], p)
            def wo_start(i):
                @pl.when(i < LAG)
                def _():
                    wo_pair(i, 0)
                    wo_pair(2 * i + LAG + 1, 1)
                @pl.when(i >= LAG)
                def _():
                    wo_pair(2 * i - LAG, 0)
                    if True:
                        j, r = (i >> 2) & 7, i & 3
                        go(wo_hbm.at[j, 3, _ds(r, 32), :], wo_buf.at[j, 3, _ds(r, 32), :], o_sem.at[jnp.maximum(j + 3, 6) if single == 4 else (6 + j if single == 8 else 6 + (j >> 2))], 1)
                    else:
                        wo_pair(i + 64, 1, True)
            def wq_start(t, p):
                s, c = t & 3, t >> 2
                go(wq_hbm.at[_ds(s, 2), _ds(c >> 2, 8), _ds(c & 3, 1024)], wq_buf.at[_ds(s, 2), _ds(c >> 2, 8), _ds(c & 3, 1024)], w_sem.at[2], p)
            def mlp_start(src, buf, i, p):
                go(src.at[:, _ds(i, 16), :], buf.at[:, _ds(i, 16), :], w_sem.at[1], p)

            NF = F2 // 16
            xc = pltpu.make_async_copy(x_hbm, x_buf, w_sem.at[0])
            if head_mode == 0:
                _loop(0, LAG, lambda t: wq_start(t, 1))
                xc.start()
                _loop(0, NF, lambda i: (mlp_start(w3t_hbm, w3_buf, i, 0), wq_start(LAG + 2 * i, 1),
                                        mlp_start(w4_hbm, w4_buf, i, 0), wq_start(LAG + 2 * i + 1, 1)))
                _loop(LAG // 2 + NF, 64, lambda i: (wq_start(2 * i, 0), wq_start(2 * i + 1, 1)))
            elif head_mode == 1:
                _loop(0, LAG // 2, lambda i: (mlp_start(w3t_hbm, w3_buf, i, 1), mlp_start(w4_hbm, w4_buf, i, 1)))
                xc.start()
                _loop(LAG // 2, NF, lambda i: (wq_start(2 * i - LAG, 0), mlp_start(w3t_hbm, w3_buf, i, 1),
                                               wq_start(2 * i - LAG + 1, 0), mlp_start(w4_hbm, w4_buf, i, 1)))
                _loop(NF - LAG // 2, 64, lambda i: (wq_start(2 * i, 0), wq_start(2 * i + 1, 1)))

            xc.wait()
            x4 = x_buf[...].astype(f32)
            x = jnp.concatenate([x4, x4], axis=0)
            xn = _layernorm(x).astype(bf16)
            xn2 = _layernorm(xn.astype(f32)).astype(bf16)
            a_buf[...] = jnp.zeros_like(a_buf)
            w3_buf[:, F2:, :] = jnp.zeros((2, FC * 128 - F2, D), bf16)
            w4_buf[:, F2:, :] = jnp.zeros((2, FC * 128 - F2, D), bf16)
            _loop(0, NP - H // 2 - 2 * FC, lambda r: kv_start(k_hbm, k_buf, k_sem, 0, r))
            wait(w3_buf.at[:, pl.ds(0, F2), :], w_sem.at[1])
            wait(w4_buf.at[:, pl.ds(0, F2), :], w_sem.at[1])
            def mlp(c, res):
                kv_start(k_hbm, k_buf, k_sem, 0, NP - H // 2 - 2 * FC + c)
                h = lax.dot_general(xn2, w3_buf[c & 1, _ds(c >> 1, 128), :], _NT, preferred_element_type=f32)
                h = jax.nn.gelu(h, approximate=True).astype(bf16)
                return res + lax.dot_general(h, w4_buf[c & 1, _ds(c >> 1, 128), :], _NN, preferred_element_type=f32)
            res = lax.fori_loop(0, 2 * FC, mlp, x + xn.astype(f32))

            wait(wq_buf, w_sem.at[2])
            def q_proj(i):
                kv_start(k_hbm, k_buf, k_sem, 0, NP - H // 2 + i)
                q = lax.dot_general(xn, wq_buf[:, :, _ds(i, 2 * DH)].reshape(D, 2 * DH), _NN, preferred_element_type=f32)
                q_buf[_ds(i, 16), :] = jnp.concatenate([q[:, :DH], q[:, DH:]], axis=0)
            _loop(0, H // 2, q_proj)

            row = lax.broadcasted_iota(jnp.int32, (8, DH), 0)
            rowu = lax.broadcasted_iota(jnp.int32, (8, CR), 0)
            def group(g):
                r0 = lax.rem(g, H // HG) * (HG * 8) + lax.div(g, H // HG)
                qg = [q_buf[pl.ds(r0 + half * 64, 8, stride=8), :].astype(bf16) for half in range(2)]
                def k_step(u, m):
                    for r in range(CR // PR):
                        kv_start(v_hbm, v_buf, v_sem, g, u * (CR // PR) + r)
                    if nocompute:
                        return m
                    ss = []
                    for half in range(2):
                        s = None
                        for j in range(8):
                            t = lax.dot_general(qg[half], k_buf[half * 8 + j, _ds(u, CR), :], _NT, preferred_element_type=f32)
                            s = t if s is None else jnp.where(rowu == j, t, s)
                        ss.append(s * scale)
                    s = jnp.concatenate(ss, axis=0)
                    s_buf[u] = s
                    return jnp.maximum(m, s)
                def k_part(w, m):
                    wait(k_buf.at[:, _ds(w, W // NW), :], k_sem.at[w])
                    return lax.fori_loop(0, NC // NW, lambda u, m: k_step(w * (NC // NW) + u, m), m)
                m = lax.fori_loop(0, NW, k_part, jnp.full((HG, CR), -jnp.inf, f32))
                m = jnp.max(m, axis=-1, keepdims=True)
                def v_step(u, c):
                    l, acc = c
                    @pl.when(g < NG - 1)
                    def _():
                        for r in range(CR // PR):
                            kv_start(k_hbm, k_buf, k_sem, g + 1, u * (CR // PR) + r)
                    @pl.when(g == NG - 1)
                    def _():
                        _loop(jnp.minimum(u * (WS * CR // 128), 64), jnp.minimum((u + 1) * (WS * CR // 128), 64), wo_start)
                    if nocompute:
                        return c
                    p = jnp.exp(s_buf[u] - m)
                    os_ = []
                    for half in range(2):
                        ph = p[half * 8:(half + 1) * 8].astype(bf16)
                        o = None
                        for j in range(8):
                            t = lax.dot_general(ph, v_buf[half * 8 + j, _ds(u, CR), :], _NN, preferred_element_type=f32)
                            o = t if o is None else jnp.where(row == j, t, o)
                        os_.append(o)
                    return l + p, acc + jnp.concatenate(os_, axis=0)
                def v_part(w, c):
                    wait(v_buf.at[:, _ds(w, W // NW), :], v_sem.at[w])
                    return lax.fori_loop(0, NC // NW, lambda u, c: v_step(w * (NC // NW) + u, c), c)
                l, acc = lax.fori_loop(0, NW, v_part, (jnp.zeros((HG, CR), f32), jnp.zeros((HG, DH), f32)))
                a_buf[pl.ds(r0, HG, stride=8), :] = acc / jnp.sum(l, axis=-1, keepdims=True)
            _loop(0, NG, group)

            def o_head(k, j, out):
                return out + lax.dot_general(a_buf[_ds(j * 4 + k, 8), :].astype(bf16), wo_buf[j, k], _NN, preferred_element_type=f32)
            def o_four(i, out):
                k, j = i >> 1, i & 1
                wait(wo_buf.at[_ds(j, 4), k], o_sem.at[i])
                for e in range(4):
                    out = o_head(k, 4 * j + e, out)
                return out
            def o_one(j, out):
                wait(wo_buf.at[j, 3], o_sem.at[(3 if single == 4 else 6) + j])
                return o_head(3, j, out)
            out = lax.fori_loop(0, 8 - single // 4, o_four, res)
            if single:
                out = lax.fori_loop(8 - single, 8, o_one, out, unroll=unroll)
            o_ref[...] = out[0:B].astype(o_ref.dtype)

        hbm = pl.BlockSpec(memory_space=pltpu.HBM)
        out = pl.pallas_call(
            kern,
            in_specs=[hbm] * 7,
            out_specs=pl.BlockSpec(memory_space=pltpu.VMEM),
            out_shape=jax.ShapeDtypeStruct((B, D), A_x.dtype),
            scratch_shapes=[
                pltpu.VMEM((B, D), bf16),
                pltpu.VMEM((HG, W, DH), bf16),
                pltpu.VMEM((HG, W, DH), bf16),
                pltpu.VMEM((8, D // 8, H * DH), bf16),
                pltpu.VMEM((8, 4, DH, D), bf16),
                pltpu.VMEM((2, FC * 128, D), bf16),
                pltpu.VMEM((2, FC * 128, D), bf16),
                pltpu.VMEM((H * 8, DH), f32),
                pltpu.VMEM((H * 8, DH), f32),
                pltpu.VMEM((NC, HG, CR), f32),
                pltpu.SemaphoreType.DMA((NW,)),
                pltpu.SemaphoreType.DMA((NW,)),
                pltpu.SemaphoreType.DMA((3,)),
                pltpu.SemaphoreType.DMA((20,)),
            ],
            compiler_params=pltpu.CompilerParams(vmem_limit_bytes=64 * 2**20, disable_bounds_checks=dbc, disable_semaphore_checks=dsc),
        )(A_x.reshape(B, D), A_k_cache.reshape(B * H, SK, DH), A_v_cache.reshape(B * H, SK, DH),
          A_wq.reshape(8, D // 8, H * DH), A_wo.reshape(8, 4, DH, D), B_w3.T.reshape(2, F2, D), B_w4.reshape(2, F2, D))
        return out.reshape(B, 1, D)
    return f


_kernel_impl = make(head_mode=1)


@jax.jit
def pallas_parallel_sum__sliding_block_cached__mixer_s_mlp__decode_kernel(
    A_x, A_k_cache, A_v_cache, A_wq, A_wo, B_x, B_w1, B_w2, B_w3, B_w4,
):
    return _kernel_impl(A_x, A_k_cache, A_v_cache, A_wq, A_wo, B_x, B_w1, B_w2, B_w3, B_w4)
```

```python
import functools

import jax
import jax.numpy as jnp
from jax import lax
from jax.experimental import pallas as pl
from jax.experimental.pallas import tpu as pltpu

_NT = (((1,), (1,)), ((), ()))
_NN = (((1,), (0,)), ((), ()))

_HG = 16
_PR = 64
_CR = 128
_LAG = 32


def _dot(a, b, dims):
    return lax.dot_general(a, b, dims, preferred_element_type=jnp.float32)


def _layernorm(x, eps=1e-5):
    d = x - jnp.mean(x, axis=-1, keepdims=True)
    return d / jnp.sqrt(jnp.mean(d * d, axis=-1, keepdims=True) + eps)


def _loop(lo, hi, fn):
    def body(i, carry):
        fn(i)
        return carry

    lax.fori_loop(lo, hi, body, 0)


def _blk(i, n):
    return pl.ds(pl.multiple_of(i * n, n), n)


def _start(src, dst, sem, queue):
    pltpu.make_async_copy(src, dst, sem).start(priority=queue)


def _wait(dst, sem):
    pltpu.make_async_copy(dst, dst, sem).wait()


def _kernel(x_hbm, k_hbm, v_hbm, wq_hbm, wo_hbm, w3t_hbm, w4_hbm, o_ref,
            x_buf, k_buf, v_buf, wq_buf, wo_buf, w3_buf, w4_buf, q_buf, a_buf, s_buf,
            k_sem, v_sem, w_sem, o_sem, *, n_heads):
    f32, bf16 = jnp.float32, jnp.bfloat16
    n_batch, d_model = x_buf.shape
    window, d_head = k_buf.shape[-2:]
    first_blk = (k_hbm.shape[-2] - window) // _PR
    n_groups = n_batch * n_heads // _HG
    f_half, f_pad = w4_hbm.shape[1], w4_buf.shape[1]

    def kv_start(src, buf, sem, g, r):
        for i, (hi, lo) in enumerate([(0, 0), (0, 2), (1, 0), (1, 2),
                                      (0, 1), (0, 3), (1, 1), (1, 3)]):
            _start(src.at[2 * g + hi, :, lo, _blk(first_blk + r, _PR), :],
                   buf.at[hi, :, lo, _blk(r, _PR), :],
                   sem.at[lax.div(r, _CR // _PR)], i % 2)

    def kv_step_start(src, buf, sem, g, u):
        for r in range(_CR // _PR):
            kv_start(src, buf, sem, g, u * (_CR // _PR) + r)

    def w3_start(i):
        _start(w3t_hbm.at[:, _blk(i, 16), :], w3_buf.at[:, _blk(i, 16), :], w_sem.at[1], 1)

    def w4_start(i):
        _start(w4_hbm.at[:, _blk(i, 16), :], w4_buf.at[:, _blk(i, 16), :], w_sem.at[2], 1)

    def wq_start(t, queue):
        idx = (_blk(t & 3, 2), _blk(t >> 4, 8), _blk((t >> 2) & 3, 1024))
        _start(wq_hbm.at[idx], wq_buf.at[idx], w_sem.at[3], queue)

    def wo_pair_start(a, queue):
        k, j2 = a >> 5, a & 3
        idx = (_blk(j2, 2), k, _blk((a >> 2) & 7, 16))
        _start(wo_hbm.at[idx], wo_buf.at[idx], o_sem.at[2 * k + (j2 >> 1)], queue)

    def wo_start(i):
        @pl.when(i < _LAG)
        def _():
            wo_pair_start(i, 0)
            wo_pair_start(2 * i + _LAG + 1, 1)

        @pl.when(i >= _LAG)
        def _():
            wo_pair_start(2 * i - _LAG, 0)
            j = (i >> 2) & 7
            idx = (j, 3, _blk(i & 3, 32))
            _start(wo_hbm.at[idx], wo_buf.at[idx], o_sem.at[jnp.maximum(j + 3, 6)], 1)

    n_f = f_half // 16
    _loop(0, _LAG // 2, lambda i: (w3_start(i), w4_start(i)))
    _start(x_hbm, x_buf, w_sem.at[0], 0)
    _loop(_LAG // 2, n_f, lambda i: (wq_start(2 * i - _LAG, 0), w3_start(i),
                                     wq_start(2 * i - _LAG + 1, 0), w4_start(i)))
    _loop(n_f - _LAG // 2, 64, lambda i: (wq_start(2 * i, 0), wq_start(2 * i + 1, 1)))

    _wait(x_buf, w_sem.at[0])
    x = x_buf[...].astype(f32)
    x = jnp.concatenate([x, x], axis=0)
    xn = _layernorm(x).astype(bf16)
    xn2 = _layernorm(xn.astype(f32)).astype(bf16)
    a_buf[...] = jnp.zeros_like(a_buf)

    n_mlp, n_q = 2 * f_pad // 128, n_heads // 2
    r_q = window // _PR - n_q
    r_mlp = r_q - n_mlp
    _loop(0, r_mlp, functools.partial(kv_start, k_hbm, k_buf, k_sem, 0))
    _wait(w3_buf.at[:, pl.ds(0, f_half), :], w_sem.at[1])
    _wait(w4_buf.at[:, pl.ds(0, f_half), :], w_sem.at[2])
    w3_buf[:, f_half:, :] = jnp.zeros((2, f_pad - f_half, d_model), bf16)
    w4_buf[:, f_half:, :] = jnp.zeros((2, f_pad - f_half, d_model), bf16)

    def mlp_step(c, res):
        kv_start(k_hbm, k_buf, k_sem, 0, r_mlp + c)
        h = _dot(xn2, w3_buf[c & 1, _blk(c >> 1, 128), :], _NT)
        h = jax.nn.gelu(h, approximate=True).astype(bf16)
        return res + _dot(h, w4_buf[c & 1, _blk(c >> 1, 128), :], _NN)

    res = lax.fori_loop(0, n_mlp, mlp_step, x + xn.astype(f32))

    _wait(wq_buf, w_sem.at[3])

    def q_step(i):
        kv_start(k_hbm, k_buf, k_sem, 0, r_q + i)
        w = wq_buf[:, :, _blk(i, 2 * d_head)].reshape(d_model, 2 * d_head)
        q = _dot(xn, w, _NN)
        q_buf[_blk(i, 16), :] = jnp.concatenate([q[:, :d_head], q[:, d_head:]], axis=0)

    _loop(0, n_q, q_step)

    def per_head_dot(lhs, buf, u, dims):
        halves = []
        for hi in range(2):
            out = None
            for j in range(8):
                t = _dot(lhs[hi], buf[hi, j // 4, j % 4, _blk(u, _CR), :], dims)
                row = lax.broadcasted_iota(jnp.int32, t.shape, 0)
                out = t if out is None else jnp.where(row == j, t, out)
            halves.append(out)
        return jnp.concatenate(halves, axis=0)

    def group(g):
        row0 = lax.rem(g, n_heads // _HG) * (8 * _HG) + lax.div(g, n_heads // _HG)
        q = [q_buf[pl.ds(row0 + 64 * hi, 8, stride=8), :].astype(bf16) for hi in range(2)]
        n_steps = window // _CR

        def k_step(u, m):
            _wait(k_buf.at[:, :, :, _blk(u, _CR), :], k_sem.at[u])
            kv_step_start(v_hbm, v_buf, v_sem, g, u)
            s = per_head_dot(q, k_buf, u, _NT) * d_head ** -0.5
            s_buf[u] = s
            return jnp.maximum(m, s)

        m = lax.fori_loop(0, n_steps, k_step, jnp.full((_HG, _CR), -jnp.inf, f32))
        m = jnp.max(m, axis=-1, keepdims=True)

        def v_step(u, carry):
            l, acc = carry
            _wait(v_buf.at[:, :, :, _blk(u, _CR), :], v_sem.at[u])

            @pl.when(g < n_groups - 1)
            def _():
                kv_step_start(k_hbm, k_buf, k_sem, g + 1, u)

            @pl.when(g == n_groups - 1)
            def _():
                _loop(0, 64 // n_steps, lambda i: wo_start(u * (64 // n_steps) + i))

            p = jnp.exp(s_buf[u] - m)
            pv = per_head_dot([p[:8].astype(bf16), p[8:].astype(bf16)], v_buf, u, _NN)
            return l + p, acc + pv

        l, acc = lax.fori_loop(
            0, n_steps, v_step,
            (jnp.zeros((_HG, _CR), f32), jnp.zeros((_HG, d_head), f32)))
        a_buf[pl.ds(row0, _HG, stride=8), :] = acc / jnp.sum(l, axis=-1, keepdims=True)

    _loop(0, n_groups, group)

    def o_head(j, k, out):
        return out + _dot(a_buf[_blk(4 * j + k, 8), :].astype(bf16), wo_buf[j, k], _NN)

    def o_four(i, out):
        k, j4 = i >> 1, i & 1
        _wait(wo_buf.at[_blk(j4, 4), k], o_sem.at[i])
        for e in range(4):
            out = o_head(4 * j4 + e, k, out)
        return out

    def o_one(j, out):
        _wait(wo_buf.at[j, 3], o_sem.at[3 + j])
        return o_head(j, 3, out)

    out = lax.fori_loop(0, 7, o_four, res)
    out = lax.fori_loop(4, 8, o_one, out)
    o_ref[...] = out[:n_batch].astype(o_ref.dtype)


@jax.jit
def pallas_parallel_sum__sliding_block_cached__mixer_s_mlp__decode_kernel(
    A_x: jax.Array,
    A_k_cache: jax.Array,
    A_v_cache: jax.Array,
    A_wq: jax.Array,
    A_wo: jax.Array,
    B_x: jax.Array,
    B_w1: jax.Array,
    B_w2: jax.Array,
    B_w3: jax.Array,
    B_w4: jax.Array,
):
    del B_x, B_w1, B_w2
    n_batch, seq, d_model = A_x.shape
    _, n_heads, kv_len, d_head = A_k_cache.shape
    d_ff = B_w3.shape[1]
    window = min(4096, max(256, kv_len // 4))
    assert (n_batch, seq, d_model, n_heads, d_head) == (4, 1, 512, 32, 128)
    assert (kv_len, d_ff) == (8192, 1376)

    f32, bf16 = jnp.float32, jnp.bfloat16
    kv_shape = (n_batch * n_heads // 8, 2, 4, kv_len, d_head)
    wq_shape = (8, d_model // 8, n_heads * d_head)
    wo_shape = (8, n_heads // 8, d_head, d_model)
    ff_shape = (2, d_ff // 2, d_model)
    ff_buf = pltpu.VMEM((2, pl.cdiv(d_ff // 2, 128) * 128, d_model), bf16)
    kv_buf = pltpu.VMEM((2, 2, 4, window, d_head), bf16)
    row_buf = pltpu.VMEM((8 * n_heads + 8, d_head), f32)

    out = pl.pallas_call(
        functools.partial(_kernel, n_heads=n_heads),
        in_specs=[pl.BlockSpec(memory_space=pltpu.HBM)] * 7,
        out_specs=pl.BlockSpec(memory_space=pltpu.VMEM),
        out_shape=jax.ShapeDtypeStruct((n_batch, d_model), A_x.dtype),
        scratch_shapes=[
            pltpu.VMEM((n_batch, d_model), bf16), kv_buf, kv_buf,
            pltpu.VMEM(wq_shape, bf16), pltpu.VMEM(wo_shape, bf16), ff_buf, ff_buf,
            row_buf, row_buf, pltpu.VMEM((window // _CR, _HG, _CR), f32),
            pltpu.SemaphoreType.DMA((window // _CR,)),
            pltpu.SemaphoreType.DMA((window // _CR,)),
            pltpu.SemaphoreType.DMA((4,)),
            pltpu.SemaphoreType.DMA((11,)),
        ],
        compiler_params=pltpu.CompilerParams(
            vmem_limit_bytes=64 * 2**20,
            disable_bounds_checks=True,
            disable_semaphore_checks=True,
        ),
    )(
        A_x.reshape(n_batch, d_model),
        A_k_cache.reshape(kv_shape),
        A_v_cache.reshape(kv_shape),
        A_wq.reshape(wq_shape),
        A_wo.reshape(wo_shape),
        B_w3.T.reshape(ff_shape),
        B_w4.reshape(ff_shape),
    )
    return out.reshape(n_batch, seq, d_model)
```
